```python
import jax
import jax.numpy as jnp

def _softmax(x, axis=-1):
    return jax.nn.softmax(x, axis=axis)
def _gelu(x):
    return jax.nn.gelu(x, approximate=True)
def _silu(x):
    return jax.nn.silu(x)
def _sigmoid(x):
    return jax.nn.sigmoid(x)
def _layernorm(x, axis=-1, eps=1e-5):
    m = jnp.mean(x, axis=axis, keepdims=True)
    v = jnp.var(x, axis=axis, keepdims=True)
    return (x - m) / jnp.sqrt(v + eps)
def _scatter_add(tgt, idx, src, axis=0):
    return tgt.at[idx].add(src)
def _segment_sum(src, seg, n):
    return jax.ops.segment_sum(src, seg, n)
class _Rng:
    def __init__(self, key):
        self._k = key
    def _next(self):
        self._k, sub = jax.random.split(self._k)
        return sub
    def normal(self, shape):
        return jax.random.normal(self._next(), shape, dtype=jnp.bfloat16)
    def randint(self, lo, hi, shape):
        return jax.random.randint(self._next(), shape, lo, hi, dtype=jnp.int32)
    def uniform(self, shape, lo=0.0, hi=1.0):
        return jax.random.uniform(self._next(), shape, jnp.bfloat16, lo, hi)
    def permutation(self, n):
        return jax.random.permutation(self._next(), n)


kernel_name = 'interleave_layers__sliding_local_dilated__glu_gated_glu__prompt'

def setup_inputs():
    _rng = _Rng(jax.random.key(int.from_bytes(__import__("os").urandom(4), "little")))
    _w = (lambda a: (lambda t: t.astype(jnp.bfloat16) if jnp.issubdtype(t.dtype, jnp.floating) else t)(jnp.asarray(a)))
    def _A_setup():
        B, S, D = 1, 2048, 576
        return {
            "x": _w((lambda *s: _rng.normal(s) * 0.05)(B, S, D)),
            "wqkv": _w((lambda *s: _rng.normal(s) * 0.05)(D, 3 * D)),
            "wo": _w((lambda *s: _rng.normal(s) * 0.05)(D, D)),
        }
    _A_in = _A_setup()

    def _B_setup():
        B, S, D, F = 1, 2048, 576, 4608
        return {
            "x": _w((lambda *s: _rng.normal(s) * 0.05)(B, S, D)),
            "w_gate": _w((lambda *s: _rng.normal(s) * 0.05)(D, F)),
            "w_up": _w((lambda *s: _rng.normal(s) * 0.05)(D, F)),
            "w_down": _w((lambda *s: _rng.normal(s) * 0.05)(F, D)),
        }
    _B_in = _B_setup()

    return {
        "A_x": _A_in["x"],
        "A_wqkv": _A_in["wqkv"],
        "A_wo": _A_in["wo"],
        "B_x": _B_in["x"],
        "B_w_gate": _B_in["w_gate"],
        "B_w_up": _B_in["w_up"],
        "B_w_down": _B_in["w_down"],
    }

def reference(A_x, A_wqkv, A_wo, B_x, B_w_gate, B_w_up, B_w_down):
    def _A_ref(x, wqkv, wo):
        B, S, D = x.shape
        H = 32; Dh = D // H
        W, dil = 8, 2
        qkv = (lambda x, *d: x.transpose(*d))((x @ wqkv).reshape(B, S, 3, H, Dh), 2, 0, 3, 1, 4)
        q, k, v = qkv[0], qkv[1], qkv[2]
        scale = Dh ** -0.5
        pos = jnp.arange(S)
        off = jnp.arange(W) * dil
        idx = pos[:, None] - off[None, :]
        mask = idx >= 0
        idx_c = jnp.where(mask, idx, 0).reshape(-1)
        kg = k[:, :, idx_c, :].reshape(B, H, S, W, Dh)
        vg = v[:, :, idx_c, :].reshape(B, H, S, W, Dh)
        logits = jnp.einsum("bhsd,bhswd->bhsw", q, kg) * scale
        logits = jnp.where(mask[None, None, :, :], logits, -1e9)
        attn = _softmax(logits, axis=-1)
        o = jnp.einsum("bhsw,bhswd->bhsd", attn, vg)
        return (lambda x, *d: x.transpose(*d))(o, 0, 2, 1, 3).reshape(B, S, D) @ wo

    def _B_ref(x, w_gate, w_up, w_down):
        g = jnp.einsum("bsd,df->bsf", x, w_gate)
        u = jnp.einsum("bsd,df->bsf", x, w_up)
        h = _sigmoid(g) * u
        return jnp.einsum("bsf,fd->bsd", h, w_down)

    x = A_x
    x = x + _A_ref(_layernorm(x, axis=-1), A_wqkv, A_wo)
    x = x + _B_ref(_layernorm(x, axis=-1), B_w_gate, B_w_up, B_w_down)
    x = x + _A_ref(_layernorm(x, axis=-1), A_wqkv, A_wo)
    x = x + _B_ref(_layernorm(x, axis=-1), B_w_gate, B_w_up, B_w_down)
    return x
```

```python
import jax
import jax.numpy as jnp
from jax import lax
import jax.experimental.pallas as pl
import jax.experimental.pallas.tpu as pltpu

S, D, F = 2048, 576, 4608
H, DH = 32, 18
WIN, DIL = 8, 2
NP = 16
L = 128
HALO = (WIN - 1) * DIL
EPS = 1e-5
SCALE = DH ** -0.5
f32, bf16, u32 = jnp.float32, jnp.bfloat16, jnp.uint32

TT = 512
FC = 1152
NFC = F // FC
NT_DIMS = (((1,), (1,)), ((), ()))


def _ln_t(x):
    m = jnp.sum(x, axis=0, keepdims=True) * (1.0 / D)
    xc = x - m
    v = jnp.sum(xc * xc, axis=0, keepdims=True) * (1.0 / D)
    return xc * lax.rsqrt(v + EPS)


def _kernel(x_hbm, wqkv_hbm, wo_hbm, wg_hbm, wu_hbm, wd_hbm, out_hbm,
            xio, wqkv_raw, wo_raw, wg, wu, wd, z, wt, wqkv_t, wo_t,
            xs, xn_t, xn, kx, vx, sems):
    cp_x = pltpu.make_async_copy(x_hbm, xio, sems.at[0])
    cp_qkv = pltpu.make_async_copy(wqkv_hbm, wqkv_raw, sems.at[1])
    cp_wo = pltpu.make_async_copy(wo_hbm, wo_raw, sems.at[2])
    glu_cps = []
    for c in range(NFC):
        for j, (src, dst) in enumerate(((wg_hbm, wg), (wu_hbm, wu), (wd_hbm, wd))):
            glu_cps.append(pltpu.make_async_copy(
                src.at[:, pl.ds(c * FC, FC)], dst.at[c], sems.at[4 + 3 * c + j]))
    cp_qkv.start()
    cp_x.start()
    cp_wo.start()

    cp_qkv.wait()
    for kt in range(5):
        kw = min(L, D - kt * L)
        w = wqkv_raw[pl.ds(kt * L, kw), :].astype(f32)
        wt[kt, :, pl.ds(0, kw)] = w.T
    for kt in range(5):
        kw = min(L, D - kt * L)
        for j in range(3):
            for d in range(DH):
                blk = wt[kt, pl.ds(j * D + d, H, stride=DH), :]
                wqkv_t[pl.ds(j * D + d * H, H), pl.ds(kt * L, kw)] = blk[:, :kw].astype(bf16)

    cp_x.wait()
    cp_wo.wait()
    for cp in glu_cps:
        cp.start()
    for c in range(3):
        rows = min(2 * L, D - c * 2 * L)
        xu = pltpu.bitcast(xio[pl.ds(c * 2 * L, rows), :], u32)
        z[c, :, pl.ds(0, rows // 2)] = xu.T
    for p in range(NP):
        parts = []
        for c in range(3):
            rows = min(2 * L, D - c * 2 * L)
            t = z[c, pl.ds(p, L, stride=NP), :].T
            parts.append(t[: rows // 2])
        xp = pltpu.bitcast(jnp.concatenate(parts, axis=0), bf16).astype(f32)
        xs[p] = xp
        xn_t[p] = _ln_t(xp).astype(bf16)

    for kt in range(5):
        kw = min(L, D - kt * L)
        wt[kt, pl.ds(0, D), pl.ds(0, kw)] = wo_raw[:, pl.ds(kt * L, kw)].astype(f32)
    for kt in range(5):
        kw = min(L, D - kt * L)
        perm = jnp.concatenate(
            [wt[kt, pl.ds(d, H, stride=DH), :] for d in range(DH)], axis=0)
        wo_t[pl.ds(kt * L, kw), :] = perm.T[:kw].astype(bf16)

    lane = lax.broadcasted_iota(jnp.int32, (H, L), 1)
    lane_d = lax.broadcasted_iota(jnp.int32, (D, L), 1)

    def attention_layer():
        def kv_body(i, carry):
            rhs = jnp.concatenate([xn_t[4 * i + j] for j in range(4)], axis=1)
            kv = jnp.dot(wqkv_t[pl.ds(D, 2 * D), :], rhs, preferred_element_type=f32)
            for j in range(4):
                kx[HALO + 4 * i + j] = kv[:D, j * L:(j + 1) * L]
                vx[HALO + 4 * i + j] = kv[D:, j * L:(j + 1) * L]
            return carry
        lax.fori_loop(0, NP // 4, kv_body, 0)

        def halo_body(i, carry):
            kx[i] = pltpu.roll(kx[i + NP], 1, 1)
            vx[i] = jnp.where(lane_d == 0, vx[HALO], pltpu.roll(vx[i + NP], 1, 1))
            return carry
        lax.fori_loop(0, HALO, halo_body, 0)

        def attend(p, q):
            logits = []
            for w in range(WIN):
                acc = None
                for d in range(DH):
                    t = q[d * H:(d + 1) * H] * kx[HALO + p - DIL * w, pl.ds(d * H, H), :]
                    acc = t if acc is None else acc + t
                lg = acc * SCALE
                if w > 0:
                    lg = jnp.where(lane * NP + (p - DIL * w) >= 0, lg, -1e9)
                logits.append(lg)
            m = logits[0]
            for lg in logits[1:]:
                m = jnp.maximum(m, lg)
            es = [jnp.exp(lg - m) for lg in logits]
            den = es[0]
            for e in es[1:]:
                den = den + e
            inv = 1.0 / den
            ps = [e * inv for e in es]
            outs = []
            for d in range(DH):
                acc = None
                for w in range(WIN):
                    t = ps[w] * vx[HALO + p - DIL * w, pl.ds(d * H, H), :]
                    acc = t if acc is None else acc + t
                outs.append(acc.astype(bf16))
            return jnp.concatenate(outs, axis=0)

        PB = 4

        def att_body(i, carry):
            for j in range(PB):
                p = PB * i + j
                q = jnp.dot(wqkv_t[pl.ds(0, D), :], xn_t[p], preferred_element_type=f32)
                o = attend(p, q)
                x = xs[p] + jnp.dot(wo_t[...], o, preferred_element_type=f32)
                xs[p] = x
                xn[pl.ds(pl.multiple_of(p * L, L), L), :] = _ln_t(x).T.astype(bf16)
            return carry
        lax.fori_loop(0, NP // PB, att_body, 0)

    def glu_layer():
        ppt = TT // L

        def body(i, carry):
            t = i // NFC
            c = i % NFC
            a = xn[pl.ds(pl.multiple_of(t * TT, TT), TT), :]
            g = jnp.dot(a, wg[c], preferred_element_type=f32)
            u = jnp.dot(a, wu[c], preferred_element_type=f32)
            h = (jax.nn.sigmoid(g) * u).astype(bf16)
            y = lax.dot_general(wd[c], h, NT_DIMS, preferred_element_type=f32)
            for j in range(ppt):
                xs[t * ppt + j] += y[:, j * L:(j + 1) * L]
            return carry
        lax.fori_loop(0, (S // TT) * NFC, body, 0)

    def layer(li, carry):
        attention_layer()

        @pl.when(li == 0)
        def _():
            for cp in glu_cps:
                cp.wait()
        glu_layer()

        @pl.when(li == 0)
        def _():
            def ln_body(p, c2):
                xn_t[p] = _ln_t(xs[p]).astype(bf16)
                return c2
            lax.fori_loop(0, NP, ln_body, 0)
        return carry
    lax.fori_loop(0, 2, layer, 0)

    for p in range(NP):
        xu = pltpu.bitcast(xs[p].astype(bf16), u32)
        for c in range(3):
            rows = min(L, D // 2 - c * L)
            t = xu[c * L:c * L + rows]
            if rows < L:
                t = jnp.concatenate([t, jnp.zeros((L - rows, L), u32)], axis=0)
            z[c, pl.ds(p, L, stride=NP), :] = t.T
    for c in range(3):
        rows = min(L, D // 2 - c * L)
        t = z[c].T[:rows]
        xio[pl.ds(c * 2 * L, 2 * rows), :] = pltpu.bitcast(t, bf16)
    cp_out = pltpu.make_async_copy(xio, out_hbm, sems.at[3])
    cp_out.start()
    cp_out.wait()


@jax.jit
def pallas_interleave_layers__sliding_local_dilated__glu_gated_glu__prompt_kernel(
    A_x, A_wqkv, A_wo, B_x, B_w_gate, B_w_up, B_w_down,
):
    del B_x
    hbm = pl.BlockSpec(memory_space=pl.ANY)
    out_t = pl.pallas_call(
        _kernel,
        out_shape=jax.ShapeDtypeStruct((D, S), bf16),
        in_specs=[hbm] * 6,
        out_specs=hbm,
        scratch_shapes=[
            pltpu.VMEM((D, S), bf16),
            pltpu.VMEM((D, 3 * D), bf16),
            pltpu.VMEM((D, D), bf16),
            pltpu.VMEM((NFC, D, FC), bf16),
            pltpu.VMEM((NFC, D, FC), bf16),
            pltpu.VMEM((NFC, D, FC), bf16),
            pltpu.VMEM((3, S, L), u32),
            pltpu.VMEM((5, 3 * D, L), f32),
            pltpu.VMEM((3 * D, D), bf16),
            pltpu.VMEM((D, D), bf16),
            pltpu.VMEM((NP, D, L), f32),
            pltpu.VMEM((NP, D, L), bf16),
            pltpu.VMEM((S, D), bf16),
            pltpu.VMEM((NP + HALO, D, L), f32),
            pltpu.VMEM((NP + HALO, D, L), f32),
            pltpu.SemaphoreType.DMA((4 + 3 * NFC,)),
        ],
        compiler_params=pltpu.CompilerParams(vmem_limit_bytes=110 * 2 ** 20),
        name="fused_layers",
    )(A_x[0].T, A_wqkv, A_wo, B_w_gate, B_w_up, B_w_down.T)
    return out_t.T[None]
```

```python
import contextlib
import jax
import jax.numpy as jnp
from jax import lax
import jax.experimental.pallas as pl
import jax.experimental.pallas.tpu as pltpu

S, D, F = 2048, 576, 4608
H, DH = 32, 18
WIN, DIL = 8, 2
NP = 16
L = 128
HALO = (WIN - 1) * DIL
EPS = 1e-5
SCALE = DH ** -0.5
f32, bf16, u32 = jnp.float32, jnp.bfloat16, jnp.uint32

FC = 512
NFC = F // FC
HG = 32
RB = 16
PLAN_B = "Q0 K0 V0 Q1 O0 K1 V1 Q2 O1 K2 Q3 O2 V2 O3 V3 K3"
PLAN_C = "Q0 Q1 Q2 O0 Q3 O1 Q4 O2 Q5 O3 Q6 O4 Q7 O5 O6 O7"
KT = 5
NT_DIMS = (((1,), (1,)), ((), ()))
PROFILE = False


def _scope(n):
    return jax.named_scope(n) if PROFILE else contextlib.nullcontext()


def _dot(a, b):
    return jnp.dot(a, b, preferred_element_type=f32)


def _dot_nt(a, b):
    return lax.dot_general(a, b, NT_DIMS, preferred_element_type=f32)


def _add(a, b):
    return (a.astype(f32) + b.astype(f32)).astype(bf16)


def _sub(a, b):
    return (a.astype(f32) - b.astype(f32)).astype(bf16)


def _tree(op, xs):
    xs = list(xs)
    while len(xs) > 1:
        xs = [op(*xs[i:i + 2]) if i + 1 < len(xs) else xs[i] for i in range(0, len(xs), 2)]
    return xs[0]


def _col_mean(x):
    acc = x[:RB]
    for r in range(RB, D, RB):
        acc = acc + x[r:r + RB]
    acc = _tree(jnp.add, [acc[r:r + 8] for r in range(0, RB, 8)])
    return jnp.sum(acc, axis=0, keepdims=True) * (1.0 / D)


def _ln_parts(x):
    xc = x - _col_mean(x)
    return xc, lax.rsqrt(_col_mean(xc * xc) + EPS)


def _ln_t(x):
    xc, rstd = _ln_parts(x)
    return xc * rstd


def _quads(m):
    n = len(m) // 2
    return [[row[j * n:(j + 1) * n] for row in m[i * n:(i + 1) * n]] for i in range(2) for j in range(2)]


def _madd(x, y):
    return [[a + b for a, b in zip(r, s)] for r, s in zip(x, y)]


def _msub(x, y):
    return [[a - b for a, b in zip(r, s)] for r, s in zip(x, y)]


def _lhs_terms(a):
    if len(a) == 1:
        return [a[0][0]]
    a11, a12, a21, a22 = _quads(a)
    terms = (_madd(a11, a22), _madd(a21, a22), a22, a11, _madd(a11, a12), _msub(a21, a11), _msub(a12, a22))
    return [t for x in terms for t in _lhs_terms(x)]


def _rhs_terms(b):
    if len(b) == 1:
        return [b[0][0]]
    b11, b12, b21, b22 = _quads(b)
    terms = (_madd(b11, b22), b11, _msub(b21, b11), _msub(b12, b22), b22, _madd(b11, b12), _madd(b21, b22))
    return [t for x in terms for t in _rhs_terms(x)]


def _combine(n, product, first=0, extra=None):
    if n == 1:
        return [[product(first)]]
    step = 7 ** (n.bit_length() - 2)
    sub = lambda k: _combine(n // 2, product, first + k * step)
    extra = extra or (lambda i, j, last: last)
    m1, m2, m4 = sub(0), sub(1), sub(2)
    c21 = _madd(extra(1, 0, m4), m2)
    m3, m5 = sub(3), sub(4)
    c12 = _madd(extra(0, 1, m5), m3)
    c22 = _madd(_msub(_madd(extra(1, 1, sub(5)), m3), m2), m1)
    c11 = _madd(_madd(_msub(extra(0, 0, sub(6)), m5), m4), m1)
    return [r + s for r, s in zip(c11, c12)] + [r + s for r, s in zip(c21, c22)]


def _pad_rows(x, rows):
    if x.shape[0] == rows:
        return x
    return jnp.concatenate([x, jnp.zeros((rows - x.shape[0], x.shape[1]), x.dtype)], axis=0)


def _kernel(x_hbm, wqkv_hbm, wo_hbm, wg_hbm, wu_hbm, wd_hbm, out_hbm,
            xio, wqkv_raw, wo_raw, wg, wu, wd, z, wt, w_att,
            xs, xn, xn_r, a_ops, xn_t, ke, ve, ko, vo, sems, wsems):
    cp_x = pltpu.make_async_copy(x_hbm, xio, sems.at[0])
    cp_qkv = pltpu.make_async_copy(wqkv_hbm, wqkv_raw, sems.at[1])
    cp_wo = pltpu.make_async_copy(wo_hbm, wo_raw, sems.at[2])

    def glu_copies(c):
        col = c * FC if isinstance(c, int) else pl.multiple_of(c * FC, FC)
        return [pltpu.make_async_copy(src.at[:, pl.ds(col, FC)], dst.at[c], wsems.at[3 * c + j])
                for j, (src, dst) in enumerate(((wg_hbm, wg), (wu_hbm, wu), (wd_hbm, wd)))]

    cp_qkv.start()
    cp_x.start()
    cp_wo.start()

    cp_qkv.wait()
    for kt in range(KT):
        kw = min(L, D - kt * L)
        wt[kt] = _pad_rows(wqkv_raw[pl.ds(kt * L, kw), :].astype(f32), L).T
    @pl.loop(0, 3)
    def _(j):
        for d in range(DH):
            blk = jnp.concatenate([wt[kt, pl.ds(j * D + d, H, stride=DH), :] for kt in range(KT)], axis=1)
            w_att[pl.ds(pl.multiple_of(j * (D // 2) + d * (H // 2), H // 2), H // 2), :] = (
                pltpu.bitcast(blk[:, :D].astype(bf16), u32))

    cp_x.wait()
    cp_wo.wait()
    for cp in glu_copies(0):
        cp.start()
    for c in range(3):
        rows = min(2 * L, D - c * 2 * L)
        xu = pltpu.bitcast(xio[pl.ds(c * 2 * L, rows), :], u32)
        z[c] = _pad_rows(xu, L).T
    @pl.loop(0, NP // 4)
    def _(i):
      for p in [4 * i + j for j in range(4)]:
        parts = []
        for c in range(3):
            rows = min(2 * L, D - c * 2 * L)
            t = z[c, pl.ds(p, L, stride=NP), :].T
            parts.append(t[: rows // 2])
        xs[p] = pltpu.bitcast(jnp.concatenate(parts, axis=0), bf16).astype(f32)

    wo = wo_raw[...].astype(f32)
    wo = jnp.concatenate([wo, jnp.zeros((D, KT * L - D), f32)], axis=1)
    for nt in range(KT):
        wt[nt, pl.ds(0, D), :] = wo[:, nt * L:(nt + 1) * L]
    for nt in range(KT):
        nw = min(L, D - nt * L)
        blk = jnp.concatenate([wt[nt, pl.ds(d, H, stride=DH), :] for d in range(DH)], axis=0)
        w_att[pl.ds((3 * D + nt * L) // 2, nw // 2), :] = pltpu.bitcast(blk.T[:nw].astype(bf16), u32)

    lane = lax.broadcasted_iota(jnp.int32, (HG, L), 1)
    lane_d = lax.broadcasted_iota(jnp.int32, (D, L), 1)

    def proj(j, rhs):
        return _dot(pltpu.bitcast(w_att[pl.ds(j * D // 2, D // 2), :], bf16), rhs)

    def norm(p):
        t = _ln_t(xs[p]).astype(bf16)
        xn_t[p] = t
        return t

    def do_o(p, o):
        x = xs[p] + proj(3, o)
        xs[p] = x
        xc, rstd = _ln_parts(x)
        rstd = jnp.broadcast_to(rstd, (L, L)).T
        xc = _pad_rows(xc, KT * L)
        rows = pl.ds(p * L if isinstance(p, int) else pl.multiple_of(p * L, L), L)
        for kt in range(4):
            xn[kt, rows, :] = xc[kt * L:(kt + 1) * L].T * rstd
        xn_r[rows, :] = (xc[4 * L:].T * rstd).astype(bf16)

    def attend(p, q, kr, vr, slot):
        outs = {}
        for g in range(0, H, HG):
            logits = [None] * WIN
            for d in range(DH):
                r = d * H + g
                for w in range(WIN):
                    t = q[r:r + HG] * kr[slot - w, pl.ds(r, HG), :]
                    logits[w] = t if d == 0 else logits[w] + t
            for w in range(WIN):
                logits[w] = logits[w] * SCALE
                if w > 0 and not (isinstance(p, int) and p - DIL * w >= 0):
                    logits[w] = jnp.where(lane * NP + (p - DIL * w) >= 0, logits[w], -1e9)
            m = _tree(jnp.maximum, logits)
            es = [jnp.exp(lg - m) for lg in logits]
            inv = pltpu.reciprocal(_tree(jnp.add, es), full_range=False)
            ps = [e * inv for e in es]
            for d in range(DH):
                r = d * H + g
                acc = None
                for w in range(WIN):
                    t = ps[w] * vr[slot - w, pl.ds(r, HG), :]
                    acc = t if acc is None else acc + t
                outs[r] = acc
        return jnp.concatenate([outs[r] for r in sorted(outs)], axis=0).astype(bf16)

    def attention_layer():
        HP = NP // 2

        def do_k(i, t, kr):
            k = proj(1, t)
            kr[HP + i] = k
            if not (isinstance(i, int) and i == 0):
                kr[i] = pltpu.roll(k, 1, 1)

        def do_v(i, t, vr):
            v = proj(2, t)
            vr[HP + i] = v
            if not (isinstance(i, int) and i == 0):
                vr[i] = jnp.where(lane_d == 0, ve[HP], pltpu.roll(v, 1, 1))

        @pl.loop(0, 2)
        def _(it):
            for i in [4 * it + j for j in range(4)]:
                t = norm(2 * i)
                do_v(i, t, ve)
                do_k(i, t, ke)

        def run(plan, i0, par, kr, vr):
            t, o = {}, {}
            for op, j in plan:
                i = i0 + j
                p = 2 * i + par
                if op == "Q":
                    o[j] = attend(p, proj(0, xn_t[p]), kr, vr, HP + i)
                elif op == "O":
                    do_o(p, o[j])
                else:
                    if j not in t:
                        t[j] = norm(p + 1)
                    (do_k if op == "K" else do_v)(i, t[j], ko if op == "K" else vo)

        @pl.loop(0, 2)
        def _(it):
            run([(s[0], int(s[1])) for s in PLAN_B.split()], it * 4, 0, ke, ve)

        run([(s[0], int(s[1])) for s in PLAN_C.split()], 0, 1, ko, vo)

    def glu_layer(li):
        TQ, FQ = S // 4, FC // 4

        @pl.loop(0, TQ // L)
        def _(i):
            r = pl.multiple_of(i * L, L)
            blocks = [[xn[k, pl.ds(t * TQ + r, L), :] for k in range(4)] for t in range(4)]
            for n, term in enumerate(_lhs_terms(blocks)):
                a_ops[n, pl.ds(r, L), :] = term.astype(bf16)

        @pl.loop(0, NFC)
        def _(c):
            @pl.when(li == 0)
            def _():
                @pl.when(c + 1 < NFC)
                def _():
                    for cp in glu_copies(c + 1):
                        cp.start()
                for cp in glu_copies(c):
                    cp.wait()

            def gu(rows, f):
                return jnp.concatenate([w[c, rows, pl.ds(f * FQ, FQ)] for w in (wg, wu)], axis=1)

            def tail(i, j, last):
                return [[_dot(xn_r[pl.ds((2 * i + t) * TQ, TQ), :][:, :D - 4 * L],
                              gu(pl.ds(4 * L, D - 4 * L), 2 * j + f)) + last[t][f]
                         for f in range(2)] for t in range(2)]

            b_ops = _rhs_terms([[gu(pl.ds(k * L, L), f).astype(f32) for f in range(4)] for k in range(4)])
            gus = _combine(4, lambda n: _dot(a_ops[n], b_ops[n].astype(bf16)), 0, tail)
            h = [[(0.5 * jnp.tanh(0.5 * v[:, :FQ]) + 0.5) * v[:, FQ:] for v in row] for row in gus]
            h = [[jnp.concatenate([jnp.concatenate(h[2 * t + a][2 * f:2 * f + 2], axis=1) for a in range(2)],
                                  axis=0) for t in range(2)] for f in range(2)]
            h_ops = _rhs_terms(h)
            w_ops = _lhs_terms([[wd[c, pl.ds(m * D // 2, D // 2), pl.ds(f * FC // 2, FC // 2)].astype(f32)
                                 for f in range(2)] for m in range(2)])
            y = _combine(2, lambda n: _dot_nt(w_ops[n].astype(bf16), h_ops[n].astype(bf16)))
            for m, t in ((1, 0), (0, 1), (1, 1), (0, 0)):
                for j in range(NP // 2):
                    xs[t * NP // 2 + j, pl.ds(m * D // 2, D // 2), :] += y[m][t][:, j * L:(j + 1) * L]

    def layer(li, carry):
        with _scope("att"):
            attention_layer()
        with _scope("glu"):
            glu_layer(li)
        return carry
    lax.fori_loop(0, 2, layer, 0)

    @pl.loop(0, NP // 4)
    def _(i):
      for p in [4 * i + j for j in range(4)]:
        xu = pltpu.bitcast(xs[p].astype(bf16), u32)
        for c in range(3):
            rows = min(L, D // 2 - c * L)
            z[c, pl.ds(p, L, stride=NP), :] = _pad_rows(xu[c * L:c * L + rows], L).T
    for c in range(3):
        rows = min(L, D // 2 - c * L)
        t = z[c].T[:rows]
        xio[pl.ds(c * 2 * L, 2 * rows), :] = pltpu.bitcast(t, bf16)
    cp_out = pltpu.make_async_copy(xio, out_hbm, sems.at[3])
    cp_out.start()
    cp_out.wait()


@jax.jit
def pallas_interleave_layers__sliding_local_dilated__glu_gated_glu__prompt_kernel(
    A_x, A_wqkv, A_wo, B_x, B_w_gate, B_w_up, B_w_down,
):
    del B_x
    hbm = pl.BlockSpec(memory_space=pl.ANY)
    out_t = pl.pallas_call(
        _kernel,
        out_shape=jax.ShapeDtypeStruct((D, S), bf16),
        in_specs=[hbm] * 6,
        out_specs=hbm,
        scratch_shapes=[
            pltpu.VMEM((D, S), bf16),
            pltpu.VMEM((D, 3 * D), bf16),
            pltpu.VMEM((D, D), bf16),
            pltpu.VMEM((NFC, D, FC), bf16),
            pltpu.VMEM((NFC, D, FC), bf16),
            pltpu.VMEM((NFC, D, FC), bf16),
            pltpu.VMEM((3, S, L), u32),
            pltpu.VMEM((KT, 3 * D, L), f32),
            pltpu.VMEM((2 * D, D), u32),
            pltpu.VMEM((NP, D, L), f32),
            pltpu.VMEM((4, S, L), f32),
            pltpu.VMEM((S, L), bf16),
            pltpu.VMEM((49, S // 4, L), bf16),
            pltpu.VMEM((NP, D, L), bf16),
            pltpu.VMEM((NP, D, L), f32),
            pltpu.VMEM((NP, D, L), f32),
            pltpu.VMEM((NP, D, L), f32),
            pltpu.VMEM((NP, D, L), f32),
            pltpu.SemaphoreType.DMA((4,)),
            pltpu.SemaphoreType.DMA((3 * NFC,)),
        ],
        compiler_params=pltpu.CompilerParams(vmem_limit_bytes=110 * 2 ** 20),
        name="fused_layers",
    )(A_x[0].T, A_wqkv, A_wo, B_w_gate, B_w_up, B_w_down.T)
    return out_t.T[None]
```

```python
import contextlib
import jax
import jax.numpy as jnp
from jax import lax
import jax.experimental.pallas as pl
import jax.experimental.pallas.tpu as pltpu

S, D, F = 2048, 576, 4608
H, DH = 32, 18
WIN, DIL = 8, 2
EPS = 1e-5
SCALE = DH ** -0.5

L = 128
NP = S // L
HP = NP // DIL
NG = H // 8
GR = D // NG
KM = 4 * L
KR = D - KM
FC = 512
NFC = F // FC
ZP = L + 8
f32, bf16, u32 = jnp.float32, jnp.bfloat16, jnp.uint32
PROFILE = False


def _scope(n):
    return jax.named_scope(n) if PROFILE else contextlib.nullcontext()


def _dot(a, b):
    return jnp.dot(a.astype(bf16), b.astype(bf16), preferred_element_type=f32)


def _dot_nt(a, b):
    return lax.dot_general(a.astype(bf16), b.astype(bf16), (((1,), (1,)), ((), ())),
                           preferred_element_type=f32)


def _words(x):
    return pltpu.bitcast(x.astype(bf16), u32)


def _halves(x):
    return pltpu.bitcast(x, bf16)


def _pad_rows(x, rows):
    if x.shape[0] == rows:
        return x
    return jnp.concatenate([x, jnp.zeros((rows - x.shape[0], x.shape[1]), x.dtype)], axis=0)


def _tree(op, xs):
    xs = list(xs)
    while len(xs) > 1:
        xs = [op(*xs[i:i + 2]) if i + 1 < len(xs) else xs[i] for i in range(0, len(xs), 2)]
    return xs[0]


def _col_mean(x):
    acc = x[:16]
    for r in range(16, D, 16):
        acc = acc + x[r:r + 16]
    return jnp.sum(acc, axis=0, keepdims=True) * (1.0 / D)


def _ln_parts(x):
    xc = x - _col_mean(x)
    return xc, lax.rsqrt(_col_mean(xc * xc) + EPS)


def _quads(block):
    return [[block(2 * i + a, 2 * j + b) for a in range(2) for b in range(2)] for i in range(2) for j in range(2)]


def _madd(x, y):
    return [a + b for a, b in zip(x, y)]


def _msub(x, y):
    return [a - b for a, b in zip(x, y)]


def _lhs7(a11, a12, a21, a22, add=jnp.add, sub=jnp.subtract):
    return [add(a11, a22), add(a21, a22), a11, a22, add(a11, a12), sub(a21, a11), sub(a12, a22)]


def _rhs7(b11, b12, b21, b22, add=jnp.add, sub=jnp.subtract):
    return [add(b11, b22), b11, sub(b12, b22), sub(b21, b11), b22, add(b11, b12), add(b21, b22)]


_OUT7 = ((1, 4, -5, 7), (3, 5), (2, 4), (1, -2, 3, 6))
_OUT10 = ((1, 4, -5, 7), (10, 3, 5, 9), (10, 2, 4, 8), (1, -2, 3, 6))


def _outputs(product, order, recipe, add=jnp.add, sub=jnp.subtract):
    m = {k: product(k) for k in order}
    out = []
    for terms in recipe:
        terms = sorted(terms, key=lambda t: -order.index(abs(t)))
        acc = m[terms[0]]
        for t in terms[1:]:
            acc = add(acc, m[t]) if t > 0 else sub(acc, m[-t])
        out.append(acc)
    return out


def _lhs10(a, r1, r2):
    t1, t2, t3, t4, t5, t6, t7 = _lhs7(*a)
    low = lax.broadcasted_iota(jnp.int32, t1.shape, 1) < L // 2
    join = lambda lo, hi: jnp.where(low, lo, hi)
    return [t1, t2, join(t3, t4), join(t4, t3), t5, join(t6, r2), join(t7, r1), join(r2, t6), join(r1, t7)]


def _rhs10(b, r1, r2):
    x1, x2, x3, x4, x5, x6, x7 = _rhs7(*[v[:L // 2] for v in b])
    b11, b12, b21, b22 = [v[L // 2:] for v in b]
    zero = jnp.zeros_like(x1)
    join = lambda lo, hi: jnp.concatenate([lo, hi], axis=0)
    return [join(x1, zero), join(x2, -b12), join(x3, b22 - b12), join(x4, b11 - b21), join(x5, -b21),
            join(x6, r2), join(x7, r1), join(r1, b11 + b12), join(r2, b21 + b22), join(zero, b12 + b21)]


_SLOT = [0, 7, 14, 23, 32, 39, 48, 57]


def _kernel(x_hbm, wqkv_hbm, wo_hbm, wg_hbm, wu_hbm, wd_hbm, out_hbm,
            xio, wqkv_raw, wo_raw, wg, wu, wd, z, wt, w_q, w_o, w_kv, w_kv_rest,
            xs, xn, xn_terms, ks, vs, v_first, sems, wsems):
    chunks = [(r, min(2 * L, D - r)) for r in range(0, D, 2 * L)]
    ktiles = [(r, min(L, D - r)) for r in range(0, D, L)]
    x_in = [pltpu.make_async_copy(x_hbm.at[pl.ds(r, n)], xio.at[pl.ds(r, n)], sems.at[c])
            for c, (r, n) in enumerate(chunks)]
    x_out = [pltpu.make_async_copy(xio.at[pl.ds(r, n)], out_hbm.at[pl.ds(r, n)], sems.at[c])
             for c, (r, n) in enumerate(chunks)]
    wo_in = pltpu.make_async_copy(wo_hbm, wo_raw, sems.at[3])
    wqkv_in = [pltpu.make_async_copy(wqkv_hbm.at[pl.ds(r, n)], wqkv_raw.at[pl.ds(r, n)], sems.at[4 + c])
               for c, (r, n) in enumerate(ktiles)]
    glu_in = [pltpu.make_async_copy(src.at[:, pl.ds(c * FC, FC)], dst.at[c], wsems.at[3 * c + j])
              for c in range(NFC)
              for j, (src, dst) in enumerate(((wg_hbm, wg), (wu_hbm, wu), (wd_hbm, wd)))]
    for cp in x_in[::-1] + [wqkv_in[kt] for kt in (0, 2, 1, 3, 4)] + [wo_in]:
        cp.start()

    for c, (r, n) in reversed(list(enumerate(chunks))):
        x_in[c].wait()
        z[pl.ds(0, S), :] = _pad_rows(_words(xio[pl.ds(r, n), :]), L).T
        for p in range(NP):
            xs[p, pl.ds(r, n), :] = _halves(z[pl.ds(p, L, stride=NP), :].T[:n // 2]).astype(f32)

    def regroup(base):
        return jnp.concatenate([wt[pl.ds(base + g * GR + d, 8, stride=DH), :]
                                for g in range(NG) for d in range(DH)], axis=0)

    def load_ktile(kt, slot):
        r, n = ktiles[kt]
        wqkv_in[kt].wait()
        wt[pl.ds(slot * 3 * D, 3 * D), :] = _pad_rows(wqkv_raw[pl.ds(r, n), :].astype(f32), L).T
        w_q[:, pl.ds(r, n)] = _words(regroup(slot * 3 * D)[:, :n])

    for kt in range(2):
        load_ktile(kt, 0)
        load_ktile(kt + 2, 1)
        terms = _lhs7(*[regroup((3 * half + j) * D) for j in (1, 2) for half in range(2)])
        for i, term in enumerate(terms):
            w_kv[i, :, pl.ds(kt * L, L)] = _words(term)
    load_ktile(4, 0)
    for j in range(2):
        w_kv_rest[j] = _words(regroup((1 + j) * D)[:, :KR])

    wo_in.wait()
    for cp in glu_in:
        cp.start()
    wo = jnp.concatenate([wo_raw[...].astype(f32), jnp.zeros((D, L - KR), f32)], axis=1)
    for nt, (r, n) in enumerate(ktiles):
        wt[pl.ds(nt * D, D), :] = wo[:, r:r + L]
        w_o[pl.ds(r // 2, n // 2), :] = _words(regroup(nt * D).T[:n])

    def attention(par):
        lane = lax.broadcasted_iota(jnp.int32, (8, L), 1)
        xt = []
        for i in range(HP):
            xc, rstd = _ln_parts(xs[2 * i + par])
            xt.append(xc * rstd)
        token0 = {}

        def kv_steps(r, n, i0, nb):
            rows = pl.ds(r, n)
            wrows = pl.ds(r // 2, n // 2)
            first = lax.broadcasted_iota(jnp.int32, (n, L), 1) == 0
            b = [jnp.concatenate(xt[i0 + t * nb:i0 + (t + 1) * nb], axis=1) for t in range(2)]
            terms = _rhs7(*[b[t][k * KM // 2:(k + 1) * KM // 2] for k in range(2) for t in range(2)])
            prod = lambda k: _dot(_halves(w_kv[k - 1, wrows, :]), terms[k - 1])
            rest = lambda m, t: _dot(_halves(w_kv_rest[m, wrows, :]), b[t][KM:])

            def put(m, t, c):
                if m == 1 and r not in token0:
                    token0[r] = jnp.where(par == 0, c[:, :L], v_first[rows, :])
                    v_first[rows, :] = token0[r]
                for j in range(nb):
                    i = i0 + t * nb + j
                    y = c[:, j * L:(j + 1) * L]
                    (ks, vs)[m][HP + i, rows, :] = y
                    if i > 0:
                        y = pltpu.roll(y, 1, 1)
                        (ks, vs)[m][i, rows, :] = jnp.where(first, token0[r], y) if m else y

            m2 = prod(2)
            yield
            m4 = prod(4)
            yield
            put(1, 0, rest(1, 0) + m4 + m2)
            m1 = prod(1)
            yield
            m3 = prod(3)
            yield
            m5 = prod(5)
            yield
            put(0, 1, rest(0, 1) + m5 + m3)
            m7 = prod(7)
            yield
            put(0, 0, rest(0, 0) + m7 - m5 + m1 + m4)
            yield
            m6 = prod(6)
            yield
            put(1, 1, rest(1, 1) + m6 + m3 + m1 - m2)
            yield

        def attend(i, g):
            q = _dot(_halves(w_q[pl.ds(g * GR // 2, GR // 2), :]), xt[i])
            logits = [None] * WIN
            for r in range(0, GR, 8):
                for w in range(WIN):
                    t = q[r:r + 8] * ks[HP + i - w, pl.ds(g * GR + r, 8), :]
                    logits[w] = t if r == 0 else logits[w] + t
            logits = [lg * SCALE if w <= i else jnp.where(lane > 0, lg * SCALE, -1e9)
                      for w, lg in enumerate(logits)]
            m = _tree(jnp.maximum, logits)
            es = [jnp.exp(lg - m) for lg in logits]
            inv = pltpu.reciprocal(_tree(jnp.add, es), full_range=False)
            ps = [e * inv for e in es]
            outs = []
            for r in range(0, GR, 8):
                acc = None
                for w in range(WIN):
                    t = ps[w] * vs[HP + i - w, pl.ds(g * GR + r, 8), :]
                    acc = t if acc is None else acc + t
                outs.append(acc)
            return jnp.concatenate(outs, axis=0)

        def project_out(i, o):
            p = 2 * i + par
            x = xs[p] + _dot(_halves(w_o[...]), jnp.concatenate(o, axis=0))
            xs[p] = x
            xc, rstd = _ln_parts(x)
            rstd = jnp.broadcast_to(rstd, (L, L)).T
            rows = pl.ds(pl.multiple_of(p * L, L), L)
            for kt in range(KM // L):
                xn[kt, rows, :] = xc[kt * L:(kt + 1) * L].T * rstd
            xn[KM // L, rows, :] = jnp.concatenate([xc[KM:], xc[KM:]], axis=0).T * rstd

        for i0 in range(0, HP, 2):
            for _ in kv_steps(0, 2 * GR, i0, 1):
                pass
        later = (None for g in (2, 3) for _ in kv_steps(g * GR, GR, 0, HP // 2))
        o = [[] for _ in range(HP)]
        next(later)
        for n in range(3 * HP):
            o[n % HP].append(attend(n % HP, n // HP))
            if n % 4:
                next(later, None)
        for i in range(HP):
            o[i].append(attend(i, 3))
            if i > 0:
                project_out(i - 1, o[i - 1])
        project_out(HP - 1, o[HP - 1])

    def glu(li):
        tq, fq = S // 4, FC // 4

        @pl.loop(0, tq // 16)
        def _(i):
            r = pl.multiple_of(i * 16, 16)
            block = lambda t, k: xn[k, pl.ds(t * tq + r, 16), :]
            r1, r2 = [block(0, 4), block(1, 4)], [block(2, 4), block(3, 4)]
            rest = {3: r1, 4: r2, 6: _msub(r2, r1), 7: _msub(r1, r2)}
            for k, a in enumerate(_lhs7(*_quads(block), _madd, _msub), 1):
                terms = _lhs10(a, *rest[k]) if k in rest else _lhs7(*a)
                for n, term in enumerate(terms):
                    xn_terms[_SLOT[k - 1] + n, pl.ds(r, 16), :] = term.astype(bf16)

        @pl.when(li == 0)
        def _():
            for cp in glu_in:
                cp.wait()

        @pl.loop(0, NFC)
        def _(c):
            def gate_up(k, f):
                rows = pl.ds(k * L, min(L, D - k * L))
                return jnp.concatenate([w[c, rows, pl.ds(f * fq, fq)] for w in (wg, wu)], axis=1).astype(f32)

            r1, r2 = [gate_up(4, 0), gate_up(4, 1)], [gate_up(4, 2), gate_up(4, 3)]
            rest = {3: r2, 4: r1, 6: r2, 7: r1}
            outer = _rhs7(*_quads(gate_up), _madd, _msub)

            def outer_product(k):
                if k in rest:
                    terms = _rhs10(outer[k - 1], *rest[k])
                    return _outputs(lambda n: _dot(xn_terms[_SLOT[k - 1] + (n - 1) % 9], terms[n - 1]),
                                    (2, 4, 10, 8, 5, 1, 7, 3, 9, 6), _OUT10)
                terms = _rhs7(*outer[k - 1])
                return _outputs(lambda n: _dot(xn_terms[_SLOT[k - 1] + n - 1], terms[n - 1]),
                                (2, 4, 1, 3, 5, 6, 7), _OUT7)

            h = []
            for quad in _outputs(outer_product, (5, 3, 2, 4, 1, 7, 6), _OUT7, _madd, _msub):
                v = [(0.5 * jnp.tanh(0.5 * gu[:, :fq]) + 0.5) * gu[:, fq:] for gu in quad]
                h.append(jnp.concatenate([jnp.concatenate(v[:2], axis=1), jnp.concatenate(v[2:], axis=1)], axis=0))
            h_terms = _rhs7(h[2], h[0], h[3], h[1])
            d_terms = _lhs7(*[wd[c, pl.ds(m * D // 2, D // 2), pl.ds(f * FC // 2, FC // 2)].astype(f32)
                              for m in range(2) for f in range(2)])
            y = _outputs(lambda n: _dot_nt(d_terms[n - 1], h_terms[n - 1]), (5, 2, 3, 1, 4, 6, 7), _OUT7)
            for m, t in ((0, 1), (1, 0), (1, 1), (0, 0)):
                for j in range(NP // 2):
                    xs[(1 - t) * NP // 2 + j, pl.ds(m * D // 2, D // 2), :] += y[2 * m + t][:, j * L:(j + 1) * L]

    @pl.loop(0, 2)
    def _(li):
        with _scope("att"):
            pl.loop(0, DIL)(attention)
        with _scope("glu"):
            glu(li)

    for c, (r, n) in enumerate(chunks):
        for p in range(NP):
            z[pl.ds(p * ZP, L), :] = _pad_rows(_words(xs[p, pl.ds(r, n), :]), L).T
        t = jnp.concatenate([z[pl.ds(l, NP, stride=ZP), :] for l in range(L)], axis=0)
        xio[pl.ds(r, n), :] = _halves(t.T[:n // 2])
        x_out[c].start()
    for cp in x_out:
        cp.wait()


@jax.jit
def pallas_interleave_layers__sliding_local_dilated__glu_gated_glu__prompt_kernel(
    A_x, A_wqkv, A_wo, B_x, B_w_gate, B_w_up, B_w_down,
):
    del B_x
    hbm = pl.BlockSpec(memory_space=pl.ANY)
    out_t = pl.pallas_call(
        _kernel,
        out_shape=jax.ShapeDtypeStruct((D, S), bf16),
        in_specs=[hbm] * 6,
        out_specs=hbm,
        scratch_shapes=[
            pltpu.VMEM((D, S), bf16),
            pltpu.VMEM((D, 3 * D), bf16),
            pltpu.VMEM((D, D), bf16),
            pltpu.VMEM((NFC, D, FC), bf16),
            pltpu.VMEM((NFC, D, FC), bf16),
            pltpu.VMEM((NFC, D, FC), bf16),
            pltpu.VMEM((NP * ZP, L), u32),
            pltpu.VMEM((6 * D, L), f32),
            pltpu.VMEM((D // 2, D), u32),
            pltpu.VMEM((D // 2, D), u32),
            pltpu.VMEM((7, D // 2, KM // 2), u32),
            pltpu.VMEM((2, D // 2, KR), u32),
            pltpu.VMEM((NP, D, L), f32),
            pltpu.VMEM((KM // L + 1, S, L), f32),
            pltpu.VMEM((_SLOT[-1], S // 4, L), bf16),
            pltpu.VMEM((2 * HP, D, L), f32),
            pltpu.VMEM((2 * HP, D, L), f32),
            pltpu.VMEM((D, L), f32),
            pltpu.SemaphoreType.DMA((9,)),
            pltpu.SemaphoreType.DMA((3 * NFC,)),
        ],
        compiler_params=pltpu.CompilerParams(vmem_limit_bytes=100 * 2 ** 20),
        name="fused_layers",
    )(A_x[0].T, A_wqkv, A_wo, B_w_gate, B_w_up, B_w_down.T)
    return out_t.T[None]
```

```python
import jax
import jax.numpy as jnp
from jax import lax
import jax.experimental.pallas as pl
import jax.experimental.pallas.tpu as pltpu

S, D, F = 2048, 576, 4608
H, DH = 32, 18
WIN, DIL = 8, 2
EPS = 1e-5
SCALE = DH ** -0.5

L = 128
NP = S // L
HP = NP // DIL
NG = H // 8
GR = D // NG
KM = 4 * L
FC = 512
NFC = F // FC
ZP = L + 8
f32, bf16, u32 = jnp.float32, jnp.bfloat16, jnp.uint32
TUNE = dict(nb=2, h=4, o10=(2, 4, 10, 8, 5, 1, 7, 3, 9, 6), rb=16)


def _dot(a, b):
    return jnp.dot(a.astype(bf16), b.astype(bf16), preferred_element_type=f32)


def _dot_nt(a, b):
    return lax.dot_general(a.astype(bf16), b.astype(bf16), (((1,), (1,)), ((), ())),
                           preferred_element_type=f32)


def _words(x):
    return pltpu.bitcast(x.astype(bf16), u32)


def _halves(x):
    return pltpu.bitcast(x, bf16)


def _pad_rows(x, rows):
    if x.shape[0] == rows:
        return x
    return jnp.concatenate([x, jnp.zeros((rows - x.shape[0], x.shape[1]), x.dtype)], axis=0)


def _tree(op, xs):
    while len(xs) > 1:
        xs = [op(a, b) for a, b in zip(xs[::2], xs[1::2])]
    return xs[0]


def _col_mean(x):
    rb = TUNE["rb"]
    acc = x[:rb]
    for r in range(rb, D, rb):
        acc = acc + x[r:r + rb]
    return jnp.sum(acc, axis=0, keepdims=True) * (1.0 / D)


def _layernorm_parts(x):
    xc = x - _col_mean(x)
    return xc, lax.rsqrt(_col_mean(xc * xc) + EPS)


_OUT7 = ((1, 4, -5, 7), (3, 5), (2, 4), (1, -2, 3, 6))
_OUT10 = ((1, 4, -5, 7), (10, 3, 5, 9), (10, 2, 4, 8), (1, -2, 3, 6))


def _lhs7(a11, a12, a21, a22, add=jnp.add, sub=jnp.subtract):
    return [add(a11, a22), add(a21, a22), a11, a22, add(a11, a12), sub(a21, a11), sub(a12, a22)]


def _rhs7(b11, b12, b21, b22, add=jnp.add, sub=jnp.subtract):
    return [add(b11, b22), b11, sub(b12, b22), sub(b21, b11), b22, add(b11, b12), add(b21, b22)]


def _lhs10(a, r1, r2):
    t1, t2, t3, t4, t5, t6, t7 = _lhs7(*a)
    low = lax.broadcasted_iota(jnp.int32, t1.shape, 1) < L // 2
    join = lambda lo, hi: jnp.where(low, lo, hi)
    return [t1, t2, join(t3, t4), join(t4, t3), t5, join(t6, r2), join(t7, r1), join(r2, t6), join(r1, t7)]


def _rhs10(b, s1, s2):
    t1, t2, t3, t4, t5, t6, t7 = _rhs7(*[v[:L // 2] for v in b])
    b11, b12, b21, b22 = [v[L // 2:] for v in b]
    zero = jnp.zeros_like(t1)
    join = lambda lo, hi: jnp.concatenate([lo, hi], axis=0)
    return [join(t1, zero), join(t2, -b12), join(t3, b22 - b12), join(t4, b11 - b21), join(t5, -b21),
            join(t6, s2), join(t7, s1), join(s1, b11 + b12), join(s2, b21 + b22), join(zero, b12 + b21)]


def _strassen_steps(product, order, recipe, emit, add=jnp.add, sub=jnp.subtract):
    m = {}
    for k in order:
        m[k] = product(k)
        for i, terms in enumerate(recipe):
            terms = sorted(terms, key=lambda t: -order.index(abs(t)))
            if abs(terms[0]) == k:
                acc = m[terms[0]]
                for t in terms[1:]:
                    acc = add(acc, m[t]) if t > 0 else sub(acc, m[-t])
                emit(i, acc)
        yield


def _strassen(product, order, recipe, *ops):
    out = [None] * 4
    for _ in _strassen_steps(product, order, recipe, out.__setitem__, *ops):
        pass
    return out


def _quads(block):
    return [[block(2 * i + a, 2 * j + b) for a in range(2) for b in range(2)]
            for i in range(2) for j in range(2)]


def _qadd(x, y):
    return [a + b for a, b in zip(x, y)]


def _qsub(x, y):
    return [a - b for a, b in zip(x, y)]


_SLOT = (0, 7, 14, 23, 32, 39, 48, 57)


def _kernel(x_hbm, wqkv_hbm, wo_hbm, wg_hbm, wu_hbm, wd_hbm, out_hbm,
            xio, wqkv_raw, wo_raw, wg, wu, wd, z, wt, w_q, w_kv, w_o,
            xs, xn, xn_terms, ks, vs, v_first, sems, wsems):
    chunks = [(r, min(2 * L, D - r)) for r in range(0, D, 2 * L)]
    tiles = [(r, min(L, D - r)) for r in range(0, D, L)]
    x_in = [pltpu.make_async_copy(x_hbm.at[pl.ds(r, n)], xio.at[pl.ds(r, n)], sems.at[c])
            for c, (r, n) in enumerate(chunks)]
    x_out = [pltpu.make_async_copy(xio.at[pl.ds(r, n)], out_hbm.at[pl.ds(r, n)], sems.at[c])
             for c, (r, n) in enumerate(chunks)]
    wo_in = pltpu.make_async_copy(wo_hbm, wo_raw, sems.at[3])
    wqkv_in = [pltpu.make_async_copy(wqkv_hbm.at[pl.ds(r, n)], wqkv_raw.at[pl.ds(r, n)], sems.at[4 + c])
               for c, (r, n) in enumerate(tiles)]
    glu_in = [pltpu.make_async_copy(src.at[:, pl.ds(c * FC, FC)], dst.at[c], wsems.at[3 * c + j])
              for c in range(NFC)
              for j, (src, dst) in enumerate(((wg_hbm, wg), (wu_hbm, wu), (wd_hbm, wd)))]
    for cp in x_in[::-1] + [wo_in] + [wqkv_in[kt] for kt in (1, 3, 4, 0, 2)]:
        cp.start()

    for c, (r, n) in reversed(list(enumerate(chunks))):
        x_in[c].wait()
        z[pl.ds(0, S), :] = _pad_rows(_words(xio[pl.ds(r, n), :]), L).T
        for p in range(NP):
            xs[p, pl.ds(r, n), :] = _halves(z[pl.ds(p, L, stride=NP), :].T[:n // 2]).astype(f32)

    def regroup(base):
        return jnp.concatenate([wt[pl.ds(base + g * GR + d, 8, stride=DH), :]
                                for g in range(NG) for d in range(DH)], axis=0)

    def twice(x):
        return x if x.shape[0] % L == 0 else jnp.concatenate([x, x[-(L // 2):]], axis=0)

    def put_terms(dst, col, terms):
        for i, term in enumerate(terms):
            dst[i, :, pl.ds(col, L)] = _words(term)

    wo_in.wait()
    wo = jnp.concatenate([wo_raw[...].astype(f32), jnp.zeros((D, L // 2), f32)], axis=1)
    parts = []
    for nt, (r, n) in enumerate(tiles):
        wt[pl.ds(nt * D, D), :] = wo[:, r:r + L]
        parts.append(twice(regroup(nt * D)).T[:n])
    wo = jnp.concatenate(parts, axis=0)
    blk = lambda m, kt: wo[m * D // 2:(m + 1) * D // 2, kt * L:(kt + 1) * L]
    put_terms(w_o, 0, _lhs7(blk(0, 0), blk(0, 2), blk(1, 0), blk(1, 2)))
    put_terms(w_o, L, _lhs10([blk(0, 1), blk(0, 3), blk(1, 1), blk(1, 3)], blk(0, 4), blk(1, 4)))

    def load_tile(kt):
        r, n = tiles[kt]
        wqkv_in[kt].wait()
        wt[pl.ds(kt * 3 * D, 3 * D), :] = twice(wqkv_raw[pl.ds(r, n), :].astype(f32)).T
        w_q[:, pl.ds(r, n)] = _words(regroup(kt * 3 * D)[:, :n])

    blk = lambda m, kt: regroup((3 * kt + 1 + m) * D)
    for kt in (1, 3, 4):
        load_tile(kt)
    put_terms(w_kv, L, _lhs10([blk(0, 1), blk(0, 3), blk(1, 1), blk(1, 3)], blk(0, 4), blk(1, 4)))
    for kt in (0, 2):
        load_tile(kt)
    for cp in glu_in:
        cp.start()
    put_terms(w_kv, 0, _lhs7(blk(0, 0), blk(0, 2), blk(1, 0), blk(1, 2)))

    def matmul_steps(w, r, n, b, emit):
        rows = pl.ds(r // 2, n // 2)
        t7 = _rhs7(*[v[kt * L:(kt + 1) * L] for kt in (0, 2) for v in b])
        t10 = _rhs10([v[kt * L:(kt + 1) * L] for kt in (1, 3) for v in b], b[0][KM:], b[1][KM:])

        def product(k):
            if k <= 7:
                return _dot(_halves(w[k - 1, rows, :]), jnp.concatenate([t7[k - 1], t10[k - 1]], axis=0))
            return _dot(_halves(w[(k - 1) % 9, rows, pl.ds(L, L)]), t10[k - 1])

        return _strassen_steps(product, TUNE["o10"], _OUT10, emit)

    def attention(par):
        lane = lax.broadcasted_iota(jnp.int32, (8, L), 1)
        xt = []
        for i in range(HP):
            xc, rstd = _layernorm_parts(xs[2 * i + par])
            xt.append(xc * rstd)
        token0 = {}

        def project_kv(r, n, nb):
            rows = pl.ds(r, n)
            first = lax.broadcasted_iota(jnp.int32, (n, L), 1) == 0
            for i0 in range(0, HP, 2 * nb):
                def emit(ci, c, i0=i0):
                    is_v, t = divmod(ci, 2)
                    if is_v and i0 + t == 0:
                        token0[r] = jnp.where(par == 0, c[:, :L], v_first[rows, :])
                        v_first[rows, :] = token0[r]
                    for j in range(nb):
                        i = i0 + t * nb + j
                        y = c[:, j * L:(j + 1) * L]
                        (ks, vs)[is_v][HP + i, rows, :] = y
                        if i > 0:
                            y = pltpu.roll(y, 1, 1)
                            (ks, vs)[is_v][i, rows, :] = jnp.where(first, token0[r], y) if is_v else y

                b = [jnp.concatenate(xt[i0 + t * nb:i0 + (t + 1) * nb], axis=1) for t in range(2)]
                yield from matmul_steps(w_kv, r, n, b, emit)

        heads = [[] for _ in range(HP)]

        def attend(i, g):
            q = _dot(_halves(w_q[pl.ds(g * GR // 2, GR // 2), :]), xt[i])
            logits = [None] * WIN
            for r in range(0, GR, 8):
                for w in range(WIN):
                    t = q[r:r + 8] * ks[HP + i - w, pl.ds(g * GR + r, 8), :]
                    logits[w] = t if r == 0 else logits[w] + t
            logits = [lg * SCALE if w <= i else jnp.where(lane > 0, lg * SCALE, -1e9)
                      for w, lg in enumerate(logits)]
            top = _tree(jnp.maximum, logits)
            es = [jnp.exp(lg - top) for lg in logits]
            inv = 1.0 / _tree(jnp.add, es)
            ps = [e * inv for e in es]
            for r in range(0, GR, 8):
                acc = None
                for w in range(WIN):
                    t = ps[w] * vs[HP + i - w, pl.ds(g * GR + r, 8), :]
                    acc = t if acc is None else acc + t
                heads[i].append(acc)

        def project_out(i0):
            halves = {}

            def emit(ci, c):
                m, t = divmod(ci, 2)
                p = 2 * (i0 + t) + par
                rows = pl.ds(m * D // 2, D // 2)
                halves[m, t] = c + xs[p, rows, :]
                xs[p, rows, :] = halves[m, t]
                if (1 - m, t) in halves:
                    xc, rstd = _layernorm_parts(jnp.concatenate([halves[0, t], halves[1, t]], axis=0))
                    rstd = jnp.broadcast_to(rstd, (L, L)).T
                    for kt, (r, n) in enumerate(tiles):
                        xn[kt, pl.ds(pl.multiple_of(p * L, L), L), :] = twice(xc[r:r + n]).T * rstd

            b = [jnp.concatenate(heads[i0 + t], axis=0) for t in range(2)]
            return matmul_steps(w_o, 0, D // 2, b, emit)

        for _ in project_kv(0, 2 * GR, 1):
            pass
        later = (None for g in (2, 3) for _ in project_kv(g * GR, GR, TUNE["nb"]))
        steps = 2 * 10 * HP // (2 * TUNE["nb"])
        next(later)
        for n in range(3 * HP):
            attend(n % HP, n // HP)
            for _ in range((n + 1) * steps // (3 * HP) - n * steps // (3 * HP)):
                next(later, None)
        later = iter(())
        for i0 in range(0, HP, 2):
            attend(i0, 3)
            for _ in range(TUNE["h"]):
                next(later, None)
            attend(i0 + 1, 3)
            for _ in later:
                pass
            later = project_out(i0)
        for _ in later:
            pass

    def glu(layer):
        tq, fq = S // 4, FC // 4

        @pl.loop(0, tq // 16)
        def _(i):
            r = pl.multiple_of(i * 16, 16)
            block = lambda t, k: xn[k, pl.ds(t * tq + r, 16), :]
            r1, r2 = [block(0, 4), block(1, 4)], [block(2, 4), block(3, 4)]
            rest = {3: r1, 4: r2, 6: _qsub(r2, r1), 7: _qsub(r1, r2)}
            for k, a in enumerate(_lhs7(*_quads(block), _qadd, _qsub), 1):
                for n, term in enumerate(_lhs10(a, *rest[k]) if k in rest else _lhs7(*a)):
                    xn_terms[_SLOT[k - 1] + n, pl.ds(r, 16), :] = term.astype(bf16)

        @pl.when(layer == 0)
        def _():
            for cp in glu_in:
                cp.wait()

        @pl.loop(0, NFC)
        def _(c):
            def gate_up(k, f):
                return jnp.concatenate([w[c, pl.ds(*tiles[k]), pl.ds(f * fq, fq)] for w in (wg, wu)],
                                       axis=1).astype(f32)

            s1, s2 = [gate_up(4, 0), gate_up(4, 1)], [gate_up(4, 2), gate_up(4, 3)]
            rest = {3: s2, 4: s1, 6: s2, 7: s1}
            outer = _rhs7(*_quads(gate_up), _qadd, _qsub)

            def outer_product(k):
                terms = _rhs10(outer[k - 1], *rest[k]) if k in rest else _rhs7(*outer[k - 1])
                product = lambda n: _dot(xn_terms[_SLOT[k - 1] + (n - 1) % 9], terms[n - 1])
                if k in rest:
                    return _strassen(product, (2, 4, 10, 8, 5, 1, 7, 3, 9, 6), _OUT10)
                return _strassen(product, (2, 4, 1, 3, 5, 6, 7), _OUT7)

            h = []
            for quad in _strassen(outer_product, (5, 3, 2, 4, 1, 7, 6), _OUT7, _qadd, _qsub):
                v = [(0.5 * jnp.tanh(0.5 * gu[:, :fq]) + 0.5) * gu[:, fq:] for gu in quad]
                h.append(jnp.concatenate([jnp.concatenate(v[:2], axis=1),
                                          jnp.concatenate(v[2:], axis=1)], axis=0))

            def emit(ci, y):
                m, t = divmod(ci, 2)
                for j in range(NP // 2):
                    xs[(1 - t) * NP // 2 + j, pl.ds(m * D // 2, D // 2), :] += y[:, j * L:(j + 1) * L]

            h_terms = _rhs7(h[2], h[0], h[3], h[1])
            d_terms = _lhs7(*[wd[c, pl.ds(m * D // 2, D // 2), pl.ds(f * FC // 2, FC // 2)].astype(f32)
                              for m in range(2) for f in range(2)])
            for _ in _strassen_steps(lambda n: _dot_nt(d_terms[n - 1], h_terms[n - 1]),
                                     (5, 2, 3, 1, 4, 6, 7), _OUT7, emit):
                pass

    @pl.loop(0, 2)
    def _(layer):
        pl.loop(0, DIL)(attention)
        glu(layer)

    for c, (r, n) in enumerate(chunks):
        for p in range(NP):
            z[pl.ds(p * ZP, L), :] = _pad_rows(_words(xs[p, pl.ds(r, n), :]), L).T
        t = jnp.concatenate([z[pl.ds(l, NP, stride=ZP), :] for l in range(L)], axis=0)
        xio[pl.ds(r, n), :] = _halves(t.T[:n // 2])
        x_out[c].start()
    for cp in x_out:
        cp.wait()


@jax.jit
def pallas_interleave_layers__sliding_local_dilated__glu_gated_glu__prompt_kernel(
    A_x: jax.Array,
    A_wqkv: jax.Array,
    A_wo: jax.Array,
    B_x: jax.Array,
    B_w_gate: jax.Array,
    B_w_up: jax.Array,
    B_w_down: jax.Array,
):
    del B_x
    hbm = pl.BlockSpec(memory_space=pl.ANY)
    out_t = pl.pallas_call(
        _kernel,
        out_shape=jax.ShapeDtypeStruct((D, S), bf16),
        in_specs=[hbm] * 6,
        out_specs=hbm,
        scratch_shapes=[
            pltpu.VMEM((D, S), bf16),
            pltpu.VMEM((D, 3 * D), bf16),
            pltpu.VMEM((D, D), bf16),
            pltpu.VMEM((NFC, D, FC), bf16),
            pltpu.VMEM((NFC, D, FC), bf16),
            pltpu.VMEM((NFC, D, FC), bf16),
            pltpu.VMEM((NP * ZP, L), u32),
            pltpu.VMEM((15 * D, L), f32),
            pltpu.VMEM((D // 2, D), u32),
            pltpu.VMEM((9, D // 2, 2 * L), u32),
            pltpu.VMEM((9, D // 4, 2 * L), u32),
            pltpu.VMEM((NP, D, L), f32),
            pltpu.VMEM((5, S, L), f32),
            pltpu.VMEM((_SLOT[-1], S // 4, L), bf16),
            pltpu.VMEM((2 * HP, D, L), f32),
            pltpu.VMEM((2 * HP, D, L), f32),
            pltpu.VMEM((D, L), f32),
            pltpu.SemaphoreType.DMA((9,)),
            pltpu.SemaphoreType.DMA((3 * NFC,)),
        ],
        compiler_params=pltpu.CompilerParams(vmem_limit_bytes=100 * 2 ** 20),
        name="fused_layers",
    )(A_x[0].T, A_wqkv, A_wo, B_w_gate, B_w_up, B_w_down.T)
    return out_t.T[None]
```

```python
import itertools

import jax
import jax.numpy as jnp
from jax import lax
import jax.experimental.pallas as pl
import jax.experimental.pallas.tpu as pltpu

S, D, F = 2048, 576, 4608
H, DH = 32, 18
WIN, DIL = 8, 2
EPS = 1e-5
SCALE = DH ** -0.5

L = 128
NP = S // L
HP = NP // DIL
NG = H // 8
GR = D // NG
KM = 4 * L
FC = 512
NFC = F // FC
ZP = L + 8
f32, bf16, u32 = jnp.float32, jnp.bfloat16, jnp.uint32


def _dot(a, b):
    return jnp.dot(a.astype(bf16), b.astype(bf16), preferred_element_type=f32)


def _dot_nt(a, b):
    return lax.dot_general(a.astype(bf16), b.astype(bf16), (((1,), (1,)), ((), ())),
                           preferred_element_type=f32)


def _words(x):
    return pltpu.bitcast(x.astype(bf16), u32)


def _halves(x):
    return pltpu.bitcast(x, bf16)


def _pad_rows(x, rows):
    if x.shape[0] == rows:
        return x
    return jnp.concatenate([x, jnp.zeros((rows - x.shape[0], x.shape[1]), x.dtype)], axis=0)


def _tree(op, xs):
    while len(xs) > 1:
        xs = [op(a, b) for a, b in zip(xs[::2], xs[1::2])]
    return xs[0]


def _col_mean(x):
    acc = x[:32]
    for r in range(32, D, 32):
        acc = acc + x[r:r + 32]
    return jnp.sum(acc, axis=0, keepdims=True) * (1.0 / D)


def _layernorm_parts(x):
    xc = x - _col_mean(x)
    return xc, lax.rsqrt(_col_mean(xc * xc) + EPS)


_OUT7 = ((1, 4, -5, 7), (3, 5), (2, 4), (1, -2, 3, 6))
_OUT10 = ((1, 4, -5, 7), (10, 3, 5, 9), (10, 2, 4, 8), (1, -2, 3, 6))


def _lhs7(a11, a12, a21, a22, add=jnp.add, sub=jnp.subtract):
    return [add(a11, a22), add(a21, a22), a11, a22, add(a11, a12), sub(a21, a11), sub(a12, a22)]


def _rhs7(b11, b12, b21, b22, add=jnp.add, sub=jnp.subtract):
    return [add(b11, b22), b11, sub(b12, b22), sub(b21, b11), b22, add(b11, b12), add(b21, b22)]


def _lhs10(a, r1, r2):
    t1, t2, t3, t4, t5, t6, t7 = _lhs7(*a)
    low = lax.broadcasted_iota(jnp.int32, t1.shape, 1) < L // 2
    join = lambda lo, hi: jnp.where(low, lo, hi)
    return [t1, t2, join(t3, t4), join(t4, t3), t5, join(t6, r2), join(t7, r1), join(r2, t6), join(r1, t7)]


def _rhs10(b, s1, s2):
    t1, t2, t3, t4, t5, t6, t7 = _rhs7(*[v[:L // 2] for v in b])
    b11, b12, b21, b22 = [v[L // 2:] for v in b]
    zero = jnp.zeros_like(t1)
    join = lambda lo, hi: jnp.concatenate([lo, hi], axis=0)
    return [join(t1, zero), join(t2, -b12), join(t3, b22 - b12), join(t4, b11 - b21), join(t5, -b21),
            join(t6, s2), join(t7, s1), join(s1, b11 + b12), join(s2, b21 + b22), join(zero, b12 + b21)]


def _strassen_steps(product, order, recipe, emit, add=jnp.add, sub=jnp.subtract):
    m = {}
    for k in order:
        m[k] = product(k)
        for i, terms in enumerate(recipe):
            terms = sorted(terms, key=lambda t: -order.index(abs(t)))
            if abs(terms[0]) == k:
                acc = m[terms[0]]
                for t in terms[1:]:
                    acc = add(acc, m[t]) if t > 0 else sub(acc, m[-t])
                emit(i, acc)
        yield


def _run(steps, n=None):
    for _ in itertools.islice(steps, n):
        pass


def _strassen(product, order, recipe, *ops):
    out = {}
    _run(_strassen_steps(product, order, recipe, out.setdefault, *ops))
    return [out[i] for i in range(4)]


def _quads(block):
    return [[block(2 * i + a, 2 * j + b) for a in range(2) for b in range(2)]
            for i in range(2) for j in range(2)]


def _qadd(x, y):
    return [a + b for a, b in zip(x, y)]


def _qsub(x, y):
    return [a - b for a, b in zip(x, y)]


_ORDER10 = (2, 4, 10, 8, 5, 1, 7, 3, 9, 6)
_SLOT = (0, 7, 14, 23, 32, 39, 48, 57)


def _kernel(x_hbm, wqkv_hbm, wo_hbm, wg_hbm, wu_hbm, wd_hbm, out_hbm,
            xio, wqkv_raw, wo_raw, wg, wu, wd, z, wt, w_q01, w_q23, w_kv, w_o,
            xs, xn, xn_terms, ks, vs, v_first, sems, wsems):
    chunks = [(r, min(2 * L, D - r)) for r in range(0, D, 2 * L)]
    tiles = [(r, min(L, D - r)) for r in range(0, D, L)]
    x_in = [pltpu.make_async_copy(x_hbm.at[pl.ds(r, n)], xio.at[pl.ds(r, n)], sems.at[c])
            for c, (r, n) in enumerate(chunks)]
    wo_in = pltpu.make_async_copy(wo_hbm, wo_raw, sems.at[3])
    wqkv_in = [pltpu.make_async_copy(wqkv_hbm.at[pl.ds(r, n)], wqkv_raw.at[pl.ds(r, n)], sems.at[4 + c])
               for c, (r, n) in enumerate(tiles)]
    glu_in = [pltpu.make_async_copy(src.at[:, pl.ds(c * FC, FC)], dst.at[c], wsems.at[3 * c + j])
              for c in range(NFC)
              for j, (src, dst) in enumerate(((wg_hbm, wg), (wu_hbm, wu), (wd_hbm, wd)))]

    def load_x(c):
        r, n = chunks[c]
        x_in[c].wait()
        z[pl.ds(0, S), :] = _pad_rows(_words(xio[pl.ds(r, n), :]), L).T
        for p in range(NP):
            xs[p, pl.ds(r, n), :] = _halves(z[pl.ds(p, L, stride=NP), :].T[:n // 2]).astype(f32)

    def regroup(base):
        return jnp.concatenate([wt[pl.ds(base + g * GR + d, 8, stride=DH), :]
                                for g in range(NG) for d in range(DH)], axis=0)

    def twice(x):
        return x if x.shape[0] % L == 0 else jnp.concatenate([x, x[-(L // 2):]], axis=0)

    def put7(dst, blk):
        for i, term in enumerate(_lhs7(blk(0, 0), blk(0, 2), blk(1, 0), blk(1, 2))):
            dst[i, :, pl.ds(0, L)] = _words(term)

    def put10(dst, blk):
        blocks = [blk(0, 1), blk(0, 3), blk(1, 1), blk(1, 3)]
        for i, term in enumerate(_lhs10(blocks, blk(0, 4), blk(1, 4))):
            dst[i, :, pl.ds(L, L)] = _words(term)

    def load_wo():
        wo_in.wait()
        wo = jnp.concatenate([wo_raw[...].astype(f32), jnp.zeros((D, L // 2), f32)], axis=1)
        parts = []
        for nt, (r, n) in enumerate(tiles):
            wt[pl.ds((15 + nt) * D, D), :] = wo[:, r:r + L]
            parts.append(twice(regroup((15 + nt) * D)).T[:n])
        wo = jnp.concatenate(parts, axis=0)
        blk = lambda m, kt: wo[m * D // 2:(m + 1) * D // 2, kt * L:(kt + 1) * L]
        put7(w_o, blk)
        put10(w_o, blk)

    def load_wqkv(kt):
        r, n = tiles[kt]
        wqkv_in[kt].wait()
        wt[pl.ds(kt * 3 * D, 3 * D), :] = twice(wqkv_raw[pl.ds(r, n), :].astype(f32)).T
        w_q23[:, pl.ds(r, n)] = _words(regroup(kt * 3 * D)[2 * GR:, :n])

    q_block = lambda m, kt: regroup(3 * kt * D)[m * GR:(m + 1) * GR]
    kv_block = lambda m, kt: regroup((3 * kt + 1 + m) * D)

    for cp in (x_in[2], wo_in, x_in[1], wqkv_in[1], wqkv_in[3], wqkv_in[4],
               x_in[0], wqkv_in[0], wqkv_in[2]):
        cp.start()
    v_first[...] = jnp.zeros_like(v_first)
    load_x(2)
    load_wo()
    load_x(1)
    for kt in (1, 3, 4):
        load_wqkv(kt)
    put10(w_kv, kv_block)
    put10(w_q01, q_block)
    load_x(0)
    for kt in (0, 2):
        load_wqkv(kt)
    for cp in glu_in:
        cp.start()
    put7(w_kv, kv_block)
    put7(w_q01, q_block)

    def matmul_steps(w, r, n, b, emit):
        rows = pl.ds(r // 2, n // 2)
        t7 = _rhs7(*[v[kt * L:(kt + 1) * L] for kt in (0, 2) for v in b])
        t10 = _rhs10([v[kt * L:(kt + 1) * L] for kt in (1, 3) for v in b], b[0][KM:], b[1][KM:])

        def product(k):
            if k <= 7:
                return _dot(_halves(w[k - 1, rows, :]), jnp.concatenate([t7[k - 1], t10[k - 1]], axis=0))
            return _dot(_halves(w[(k - 1) % 9, rows, pl.ds(L, L)]), t10[k - 1])

        return _strassen_steps(product, _ORDER10, _OUT10, emit)

    def attention(par):
        lane = lax.broadcasted_iota(jnp.int32, (8, L), 1)
        xt = []
        for i in range(HP):
            xc, rstd = _layernorm_parts(xs[2 * i + par])
            xt.append(xc * rstd)
        token0 = {}

        def project_kv(r, n):
            rows = pl.ds(r, n)
            first = lax.broadcasted_iota(jnp.int32, (n, L), 1) == 0
            for i0 in range(0, HP, 2):
                def emit(ci, y, i0=i0):
                    is_v, i = ci // 2, i0 + ci % 2
                    (ks, vs)[is_v][HP + i, rows, :] = y
                    if i > 0:
                        y = pltpu.roll(y, 1, 1)
                        (ks, vs)[is_v][i, rows, :] = jnp.where(first, token0[r], y) if is_v else y
                    elif is_v:
                        token0[r] = jnp.where(par == 0, y, v_first[rows, :])
                        v_first[rows, :] = token0[r]

                yield from matmul_steps(w_kv, r, n, xt[i0:i0 + 2], emit)

        heads = [{} for _ in range(HP)]

        def attend(i, g, q=None):
            if q is None:
                q = _dot(_halves(w_q23[pl.ds((g - 2) * GR // 2, GR // 2), :]), xt[i])
            logits = [None] * WIN
            for r in range(0, GR, 8):
                for w in range(WIN):
                    t = q[r:r + 8] * ks[HP + i - w, pl.ds(g * GR + r, 8), :]
                    logits[w] = t if r == 0 else logits[w] + t
            logits = [lg * SCALE if w <= i else jnp.where(lane > 0, lg * SCALE, -1e9)
                      for w, lg in enumerate(logits)]
            top = _tree(jnp.maximum, logits)
            es = [jnp.exp(lg - top) for lg in logits]
            inv = 1.0 / _tree(jnp.add, es)
            ps = [e * inv for e in es]
            for r in range(0, GR, 8):
                acc = None
                for w in range(WIN):
                    t = ps[w] * vs[HP + i - w, pl.ds(g * GR + r, 8), :]
                    acc = t if acc is None else acc + t
                heads[i][g * GR + r] = acc

        def project_out(i0):
            halves = {}

            def emit(ci, c):
                m, t = divmod(ci, 2)
                p = 2 * (i0 + t) + par
                rows = pl.ds(m * D // 2, D // 2)
                halves[m, t] = c + xs[p, rows, :]
                xs[p, rows, :] = halves[m, t]
                if (1 - m, t) in halves:
                    xc, rstd = _layernorm_parts(jnp.concatenate([halves[0, t], halves[1, t]], axis=0))
                    rstd = jnp.broadcast_to(rstd, (L, L)).T
                    for kt, (r, n) in enumerate(tiles):
                        xn[kt, pl.ds(pl.multiple_of(p * L, L), L), :] = twice(xc[r:r + n]).T * rstd

            b = [jnp.concatenate([heads[i0 + t][r] for r in range(0, D, 8)], axis=0) for t in range(2)]
            return matmul_steps(w_o, 0, D // 2, b, emit)

        def attend_early():
            for i0 in range(0, HP, 2):
                yield from matmul_steps(w_q01, 0, GR, xt[i0:i0 + 2],
                                        lambda ci, q, i0=i0: attend(i0 + ci % 2, ci // 2, q))
            for i in range(HP):
                attend(i, 2)
                yield from range(3)

        _run(project_kv(0, 2 * GR))
        filler = itertools.chain(project_kv(2 * GR, GR), project_kv(3 * GR, GR))
        for n, _ in enumerate(attend_early()):
            _run(filler, 2 if n % 4 == 3 else 1)
        for i0 in range(0, HP, 2):
            attend(i0, 3)
            _run(filler, 4)
            attend(i0 + 1, 3)
            _run(filler)
            filler = project_out(i0)
        _run(filler)

    def glu(layer):
        tq, fq = S // 4, FC // 4

        @pl.loop(0, tq // 16)
        def _(i):
            r = pl.multiple_of(i * 16, 16)
            block = lambda t, k: xn[k, pl.ds(t * tq + r, 16), :]
            r1, r2 = [block(0, 4), block(1, 4)], [block(2, 4), block(3, 4)]
            rest = {3: r1, 4: r2, 6: _qsub(r2, r1), 7: _qsub(r1, r2)}
            for k, a in enumerate(_lhs7(*_quads(block), _qadd, _qsub), 1):
                for n, term in enumerate(_lhs10(a, *rest[k]) if k in rest else _lhs7(*a)):
                    xn_terms[_SLOT[k - 1] + n, pl.ds(r, 16), :] = term.astype(bf16)

        @pl.when(layer == 0)
        def _():
            for cp in glu_in:
                cp.wait()

        @pl.loop(0, NFC)
        def _(c):
            def gate_up(k, f):
                return jnp.concatenate([w[c, pl.ds(*tiles[k]), pl.ds(f * fq, fq)] for w in (wg, wu)],
                                       axis=1).astype(f32)

            s1, s2 = [gate_up(4, 0), gate_up(4, 1)], [gate_up(4, 2), gate_up(4, 3)]
            rest = {3: s2, 4: s1, 6: s2, 7: s1}
            outer = _rhs7(*_quads(gate_up), _qadd, _qsub)

            def outer_product(k):
                terms = _rhs10(outer[k - 1], *rest[k]) if k in rest else _rhs7(*outer[k - 1])
                product = lambda n: _dot(xn_terms[_SLOT[k - 1] + (n - 1) % 9], terms[n - 1])
                if k in rest:
                    return _strassen(product, _ORDER10, _OUT10)
                return _strassen(product, (2, 4, 1, 3, 5, 6, 7), _OUT7)

            h = []
            for quad in _strassen(outer_product, (5, 3, 2, 4, 1, 7, 6), _OUT7, _qadd, _qsub):
                v = [(0.5 * jnp.tanh(0.5 * gu[:, :fq]) + 0.5) * gu[:, fq:] for gu in quad]
                h.append(jnp.concatenate([jnp.concatenate(v[:2], axis=1),
                                          jnp.concatenate(v[2:], axis=1)], axis=0))

            def emit(ci, y):
                m, t = divmod(ci, 2)
                for j in range(NP // 2):
                    xs[(1 - t) * NP // 2 + j, pl.ds(m * D // 2, D // 2), :] += y[:, j * L:(j + 1) * L]

            h_terms = _rhs7(h[2], h[0], h[3], h[1])
            d_terms = _lhs7(*[wd[c, pl.ds(m * D // 2, D // 2), pl.ds(f * FC // 2, FC // 2)].astype(f32)
                              for m in range(2) for f in range(2)])
            _run(_strassen_steps(lambda n: _dot_nt(d_terms[n - 1], h_terms[n - 1]),
                                 (5, 2, 3, 1, 4, 6, 7), _OUT7, emit))

    @pl.loop(0, 2)
    def _(layer):
        pl.loop(0, DIL)(attention)
        glu(layer)

    x_out = []
    for r, n in chunks:
        for p in range(NP):
            z[pl.ds(p * ZP, L), :] = _pad_rows(_words(xs[p, pl.ds(r, n), :]), L).T
        for l0 in range(0, L, 32):
            t = jnp.concatenate([z[pl.ds(l, NP, stride=ZP), :] for l in range(l0, l0 + 32)], axis=0)
            part = (pl.ds(r, n), pl.ds(l0 * NP, 32 * NP))
            xio[part] = _halves(t.T[:n // 2])
            x_out.append(pltpu.make_async_copy(xio.at[part], out_hbm.at[part], wsems.at[len(x_out)]))
            x_out[-1].start()
    for cp in x_out:
        cp.wait()


@jax.jit
def pallas_interleave_layers__sliding_local_dilated__glu_gated_glu__prompt_kernel(
    A_x: jax.Array,
    A_wqkv: jax.Array,
    A_wo: jax.Array,
    B_x: jax.Array,
    B_w_gate: jax.Array,
    B_w_up: jax.Array,
    B_w_down: jax.Array,
):
    del B_x
    hbm = pl.BlockSpec(memory_space=pl.ANY)
    out_t = pl.pallas_call(
        _kernel,
        out_shape=jax.ShapeDtypeStruct((D, S), bf16),
        in_specs=[hbm] * 6,
        out_specs=hbm,
        scratch_shapes=[
            pltpu.VMEM((D, S), bf16),
            pltpu.VMEM((D, 3 * D), bf16),
            pltpu.VMEM((D, D), bf16),
            pltpu.VMEM((NFC, D, FC), bf16),
            pltpu.VMEM((NFC, D, FC), bf16),
            pltpu.VMEM((NFC, D, FC), bf16),
            pltpu.VMEM((NP * ZP + L, L), u32),
            pltpu.VMEM((20 * D + L, L), f32),
            pltpu.VMEM((9, GR // 2, 2 * L), u32),
            pltpu.VMEM((GR, D), u32),
            pltpu.VMEM((9, D // 2, 2 * L), u32),
            pltpu.VMEM((9, D // 4, 2 * L), u32),
            pltpu.VMEM((NP, D, L), f32),
            pltpu.VMEM((5, S, L), f32),
            pltpu.VMEM((_SLOT[-1], S // 4, L), bf16),
            pltpu.VMEM((2 * HP, D, L), f32),
            pltpu.VMEM((2 * HP, D, L), f32),
            pltpu.VMEM((D, L), f32),
            pltpu.SemaphoreType.DMA((9,)),
            pltpu.SemaphoreType.DMA((3 * NFC,)),
        ],
        compiler_params=pltpu.CompilerParams(vmem_limit_bytes=100 * 2 ** 20),
        name="fused_layers",
    )(A_x.reshape(S, D).T, A_wqkv, A_wo, B_w_gate, B_w_up, B_w_down.T)
    return out_t.T.reshape(1, S, D)
```
